```python
import jax
import jax.numpy as jnp

def _softmax(x, axis=-1):
    return jax.nn.softmax(x, axis=axis)
def _gelu(x):
    return jax.nn.gelu(x, approximate=True)
def _silu(x):
    return jax.nn.silu(x)
def _sigmoid(x):
    return jax.nn.sigmoid(x)
def _layernorm(x, axis=-1, eps=1e-5):
    m = jnp.mean(x, axis=axis, keepdims=True)
    v = jnp.var(x, axis=axis, keepdims=True)
    return (x - m) / jnp.sqrt(v + eps)
def _scatter_add(tgt, idx, src, axis=0):
    return tgt.at[idx].add(src)
def _segment_sum(src, seg, n):
    return jax.ops.segment_sum(src, seg, n)
class _Rng:
    def __init__(self, key):
        self._k = key
    def _next(self):
        self._k, sub = jax.random.split(self._k)
        return sub
    def normal(self, shape):
        return jax.random.normal(self._next(), shape, dtype=jnp.bfloat16)
    def randint(self, lo, hi, shape):
        return jax.random.randint(self._next(), shape, lo, hi, dtype=jnp.int32)
    def uniform(self, shape, lo=0.0, hi=1.0):
        return jax.random.uniform(self._next(), shape, jnp.bfloat16, lo, hi)
    def permutation(self, n):
        return jax.random.permutation(self._next(), n)


kernel_name = 'recurrent_scan__sliding_block_cached__glu_gated_swiglu__decode'

def setup_inputs():
    _rng = _Rng(jax.random.key(int.from_bytes(__import__("os").urandom(4), "little")))
    _w = (lambda a: (lambda t: t.astype(jnp.bfloat16) if jnp.issubdtype(t.dtype, jnp.floating) else t)(jnp.asarray(a)))
    def _A_setup():
        B, Sq, D = 1, 1, 640
        Hq, Hkv, Sk, Dh = 32, 32, 32768, 192
        assert Hq % Hkv == 0, (Hq, Hkv)
        return {
            "x": _w((lambda *s: _rng.normal(s) * 0.05)(B, Sq, D)),
            "k_cache": _w((lambda *s: _rng.normal(s) * 0.05)(B, Hkv, Sk, Dh)),
            "v_cache": _w((lambda *s: _rng.normal(s) * 0.05)(B, Hkv, Sk, Dh)),
            "wq": _w((lambda *s: _rng.normal(s) * 0.05)(D, Hq * Dh) * (D ** -0.5)),
            "wo": _w((lambda *s: _rng.normal(s) * 0.05)(Hq * Dh, D) * ((Hq * Dh) ** -0.5)),
        }
    _A_in = _A_setup()

    def _B_setup():
        B, S, D, F = 1, 1, 640, 1536
        return {
            "x": _w((lambda *s: _rng.normal(s) * 0.05)(B, S, D)),
            "w1": _w((lambda *s: _rng.normal(s) * 0.05)(D, F) * (2.0 / D) ** 0.5),
            "w3": _w((lambda *s: _rng.normal(s) * 0.05)(D, F) * (2.0 / D) ** 0.5),
            "w2": _w((lambda *s: _rng.normal(s) * 0.05)(F, D) * (2.0 / F) ** 0.5),
        }
    _B_in = _B_setup()

    return {
        "A_x": _A_in["x"],
        "A_k_cache": _A_in["k_cache"],
        "A_v_cache": _A_in["v_cache"],
        "A_wq": _A_in["wq"],
        "A_wo": _A_in["wo"],
        "B_x": _B_in["x"],
        "B_w1": _B_in["w1"],
        "B_w3": _B_in["w3"],
        "B_w2": _B_in["w2"],
    }

def reference(A_x, A_k_cache, A_v_cache, A_wq, A_wo, B_x, B_w1, B_w3, B_w2):
    def _A_ref(x, k_cache, v_cache, wq, wo):
        B, Sq, D = x.shape
        Hq, Dh = 32, 192
        Hkv, Sk = k_cache.shape[1], k_cache.shape[2]
        W = min(4096, max(256, Sk // 4))
        rep = Hq // Hkv
        q = (lambda x, *d: x.transpose(*d))((x @ wq).reshape(B, Sq, Hq, Dh), 0, 2, 1, 3)
        k = jnp.repeat(k_cache[:, :, Sk - W:, :], rep, axis=1)
        v = jnp.repeat(v_cache[:, :, Sk - W:, :], rep, axis=1)
        scores = jnp.einsum("bhqd,bhkd->bhqk", q, k) * (Dh ** -0.5)
        p = _softmax(scores, axis=-1)
        o = jnp.einsum("bhqk,bhkd->bhqd", p, v)
        return (lambda x, *d: x.transpose(*d))(o, 0, 2, 1, 3).reshape(B, Sq, Hq * Dh) @ wo

    def _B_ref(x, w1, w3, w2):
        gate = jnp.einsum("bsd,df->bsf", x, w1)
        up = jnp.einsum("bsd,df->bsf", x, w3)
        h = _silu(gate) * up
        out = jnp.einsum("bsf,fd->bsd", h, w2)
        return out

    x = A_x
    xn = _layernorm(x, axis=-1)
    s = _A_ref(xn, A_k_cache, A_v_cache, A_wq, A_wo)
    g = _silu(_B_ref(xn, B_w1, B_w3, B_w2))
    return x + s * g
```

```python
import jax
import jax.numpy as jnp
from jax import lax
import jax.experimental.pallas as pl
import jax.experimental.pallas.tpu as pltpu

_HQ = 32
_DH = 192
_ROWS = 8
_EPS = 1e-5


def _silu(z):
    return z / (1.0 + jnp.exp(-z))


def _kernel(x_hbm, k_hbm, v_hbm, wq_hbm, wo_hbm, w1_hbm, w3_hbm, w2_hbm,
            o_ref,
            x_buf, wq_buf, k_buf, v_buf, wo_buf, w1_buf, w3_buf, w2_buf,
            q_buf, sems, *, window):
    d_model = wq_hbm.shape[0]
    d_ff = w1_hbm.shape[1]
    seq = k_hbm.shape[3]
    pair = 2 * _DH
    n_pairs = _HQ // 2
    s0 = seq - window
    half = window // 2
    scale = _DH ** -0.5
    sem_x, sem_wq, sem_k, sem_v, sem_w13, sem_w2 = (sems.at[i] for i in range(6))

    def copy(src, dst, sem, queue):
        pltpu.make_async_copy(src, dst, sem).start(priority=queue)

    def wait_all(buf, sem):
        pltpu.make_async_copy(buf, buf, sem).wait()

    def start_cache(hbm, buf, sem, p):
        def body(r, carry):
            r0 = pl.multiple_of(r * 8, 8)
            for c in range(2):
                for j in range(2):
                    copy(hbm.at[0, 2 * p + j, pl.ds(r0, 8), pl.ds(s0 + c * half, half)],
                         buf.at[pl.ds(j * _DH + r0, 8), pl.ds(c * half, half)],
                         sem, j)
            return carry
        lax.fori_loop(0, _DH // 8, body, None)

    def start_rows(hbm, row0, buf, sem, rows):
        def body(i, carry):
            for j in range(2):
                r0 = pl.multiple_of((2 * i + j) * rows, 8)
                copy(hbm.at[pl.ds(row0 + r0, rows), :], buf.at[pl.ds(r0, rows), :], sem, j)
            return carry
        lax.fori_loop(0, buf.shape[0] // (2 * rows), body, None)

    def start_wq():
        cols = 2048
        def body(i, carry):
            for c in range(wq_buf.shape[1] // cols):
                for j in range(2):
                    r0 = pl.multiple_of((2 * i + j) * 8, 8)
                    copy(wq_hbm.at[pl.ds(r0, 8), pl.ds(c * cols, cols)],
                         wq_buf.at[pl.ds(r0, 8), pl.ds(c * cols, cols)], sem_wq, j)
            return carry
        lax.fori_loop(0, d_model // 16, body, None)

    def start_w13():
        def body(i, carry):
            r0 = pl.multiple_of(i * 8, 8)
            copy(w1_hbm.at[pl.ds(r0, 8), :], w1_buf.at[pl.ds(r0, 8), :], sem_w13, 0)
            copy(w3_hbm.at[pl.ds(r0, 8), :], w3_buf.at[pl.ds(r0, 8), :], sem_w13, 1)
            return carry
        lax.fori_loop(0, d_model // 8, body, None)

    def start_v(p):
        start_rows(wo_hbm, pl.multiple_of(p * pair, pair), wo_buf, sem_v, 24)
        start_cache(v_hbm, v_buf, sem_v, p)

    row = lax.broadcasted_iota(jnp.int32, (_ROWS, pair), 0)
    lane = lax.broadcasted_iota(jnp.int32, (_ROWS, pair), 1)
    own = (lane >= row * _DH) & (lane < (row + 1) * _DH)

    x_copy = pltpu.make_async_copy(x_hbm.at[0], x_buf, sem_x)
    x_copy.start()
    start_wq()
    start_cache(k_hbm, k_buf, sem_k, 0)

    x_copy.wait()
    x = x_buf[...].astype(jnp.float32)
    mean = jnp.mean(x, axis=-1, keepdims=True)
    xc = x - mean
    var = jnp.mean(xc * xc, axis=-1, keepdims=True)
    xn = xc / jnp.sqrt(var + _EPS)
    xn = jnp.broadcast_to(xn, (_ROWS, d_model)).astype(jnp.bfloat16)

    wait_all(wq_buf, sem_wq)
    for p in range(n_pairs):
        q = jnp.dot(xn, wq_buf[:, p * pair:(p + 1) * pair],
                    preferred_element_type=jnp.float32)
        q_buf[p] = jnp.where(own, q, 0.0)

    def pair_step(p, acc):
        start_v(p)

        wait_all(k_buf, sem_k)
        s = jnp.dot(q_buf[p].astype(jnp.bfloat16), k_buf[...],
                    preferred_element_type=jnp.float32) * scale
        e = jnp.exp(s - jnp.max(s, axis=-1, keepdims=True))
        denom = jnp.sum(e, axis=-1, keepdims=True)
        e = e.astype(jnp.bfloat16)

        @pl.when(p + 1 < n_pairs)
        def _():
            start_cache(k_hbm, k_buf, sem_k, p + 1)

        @pl.when(p + 1 == n_pairs)
        def _():
            start_w13()

        wait_all(wo_buf, sem_v)
        wait_all(v_buf, sem_v)
        o = lax.dot_general(e, v_buf[...], (((1,), (1,)), ((), ())),
                            preferred_element_type=jnp.float32)
        o = jnp.where(own, o / denom, 0.0).astype(jnp.bfloat16)
        return acc + jnp.dot(o, wo_buf[...], preferred_element_type=jnp.float32)

    acc = lax.fori_loop(0, n_pairs, pair_step,
                        jnp.zeros((_ROWS, d_model), jnp.float32))
    attn = jnp.sum(acc, axis=0, keepdims=True)

    start_rows(w2_hbm, 0, w2_buf, sem_w2, 24)
    wait_all(w1_buf, sem_w13)
    wait_all(w3_buf, sem_w13)
    gate = jnp.dot(xn, w1_buf[...], preferred_element_type=jnp.float32)
    up = jnp.dot(xn, w3_buf[...], preferred_element_type=jnp.float32)
    h = (_silu(gate) * up).astype(jnp.bfloat16)
    wait_all(w2_buf, sem_w2)
    ffn = jnp.dot(h, w2_buf[...], preferred_element_type=jnp.float32)
    g = _silu(ffn[0:1, :])

    o_ref[0] = (x + attn * g).astype(o_ref.dtype)


@jax.jit
def pallas_recurrent_scan__sliding_block_cached__glu_gated_swiglu__decode_kernel(
    A_x: jax.Array,
    A_k_cache: jax.Array,
    A_v_cache: jax.Array,
    A_wq: jax.Array,
    A_wo: jax.Array,
    B_x: jax.Array,
    B_w1: jax.Array,
    B_w3: jax.Array,
    B_w2: jax.Array,
):
    del B_x
    batch, sq, d_model = A_x.shape
    _, hkv, seq, dh = A_k_cache.shape
    assert (batch, sq, hkv, dh) == (1, 1, _HQ, _DH)
    d_ff = B_w1.shape[1]
    window = min(4096, max(256, seq // 4))

    k_t = jnp.swapaxes(A_k_cache, 2, 3)
    v_t = jnp.swapaxes(A_v_cache, 2, 3)

    def kernel(*refs):
        _kernel(*refs, window=window)

    bf16 = jnp.bfloat16
    hbm = pl.BlockSpec(memory_space=pltpu.HBM)
    return pl.pallas_call(
        kernel,
        out_shape=jax.ShapeDtypeStruct(A_x.shape, A_x.dtype),
        in_specs=[hbm] * 8,
        out_specs=pl.BlockSpec(memory_space=pltpu.VMEM),
        scratch_shapes=[
            pltpu.VMEM((1, d_model), bf16),
            pltpu.VMEM((d_model, _HQ * _DH), bf16),
            pltpu.VMEM((2 * _DH, window), bf16),
            pltpu.VMEM((2 * _DH, window), bf16),
            pltpu.VMEM((2 * _DH, d_model), bf16),
            pltpu.VMEM((d_model, d_ff), bf16),
            pltpu.VMEM((d_model, d_ff), bf16),
            pltpu.VMEM((d_ff, d_model), bf16),
            pltpu.VMEM((_HQ // 2, _ROWS, 2 * _DH), jnp.float32),
            pltpu.SemaphoreType.DMA((6,)),
        ],
        compiler_params=pltpu.CompilerParams(
            vmem_limit_bytes=64 * 1024 * 1024,
        ),
    )(A_x, k_t, v_t, A_wq, A_wo, B_w1, B_w3, B_w2)
```

```python
import jax
import jax.numpy as jnp
from jax import lax
import jax.experimental.pallas as pl
import jax.experimental.pallas.tpu as pltpu

_HQ = 32
_DH = 192
_ROWS = 8
_LANES = 128
_STEPS = 8
_EPS = 1e-5


def _silu(z):
    return z / (1.0 + jnp.exp(-z))


def _dot(a, b):
    return jnp.dot(a, b, preferred_element_type=jnp.float32)


def _dot_t(a, b):
    return lax.dot_general(a, b, (((1,), (1,)), ((), ())),
                           preferred_element_type=jnp.float32)


def _kernel(x_hbm, k_hbm, v_hbm, wq_hbm, wo_hbm, w1_hbm, w3_hbm, w2_hbm,
            o_ref,
            x_buf, wq_buf, k_buf, v_buf, wo_buf, w1_buf, w3_buf, w2_buf,
            q_buf, s_buf, a_buf, sems, k_sems, v_sems, wo_sems, *, window):
    d_model = x_buf.shape[1]
    seq = k_hbm.shape[3]
    pair = 2 * _DH
    n_pairs = _HQ // 2
    n_tiles = window // _LANES
    step_tiles = n_tiles // _STEPS
    scale = _DH ** -0.5
    sem_x, sem_wq, sem_ffn = (sems.at[i] for i in range(3))
    wo_slabs, wo_rows, _ = wo_buf.shape
    wo_chunks = wo_rows // _LANES - 1

    def copy(src, dst, sem, queue):
        pltpu.make_async_copy(src, dst, sem).start(priority=queue)

    def mirror(hbm, buf, idx, sem, queue):
        copy(hbm.at[idx], buf.at[idx], sem, queue)

    def wait_all(buf, sem):
        pltpu.make_async_copy(buf, buf, sem).wait()

    def loop(n, body):
        lax.fori_loop(0, n, lambda i, c: body(i), None)

    def rows8(r):
        return pl.ds(pl.multiple_of(r, 8), 8)

    def start_cache(hbm, buf, buf_sems, p, step, n_steps):
        rows = _DH // 2
        half = n_steps // 2
        tiles = n_tiles // half
        slot = p % 2
        r0 = pl.multiple_of((step // half) * rows, rows)
        for c in range(tiles):
            t = (step % half) * tiles + c
            c0 = pl.multiple_of(seq - window + t * _LANES, _LANES)
            for j in range(2):
                copy(hbm.at[0, 2 * p + j, pl.ds(r0, rows), pl.ds(c0, _LANES)],
                     buf.at[slot, t, pl.ds(j * _DH + r0, rows), :],
                     buf_sems.at[slot], j)

    def start_wq():
        slabs = wq_buf.shape[0] // 2
        def body(i):
            for c in range(0, wq_buf.shape[2], 512):
                for j in range(2):
                    mirror(wq_hbm, wq_buf,
                           (pl.ds(j * slabs, slabs), rows8(i * 8), pl.ds(c, 512)),
                           sem_wq, j)
        loop(wq_buf.shape[1] // 8, body)

    def start_ffn():
        cols = range(0, w1_buf.shape[2], 512)
        n_iter = w1_buf.shape[1] // 16
        def body(i):
            n = 0
            for r in (0, 8):
                for c in cols:
                    idx = (slice(None), rows8(i * 16 + r), pl.ds(c, 512))
                    mirror(w1_hbm, w1_buf, idx, sem_ffn, n % 2)
                    mirror(w3_hbm, w3_buf, idx, sem_ffn, 1 - n % 2)
                    mirror(w2_hbm, w2_buf,
                           (slice(None), rows8((i * 2 * len(cols) + n) * 8)),
                           sem_ffn, n % 2)
                    n += 1
        loop(n_iter, body)
        for n in range(n_iter * 2 * len(cols), w2_buf.shape[1] // 8):
            mirror(w2_hbm, w2_buf, (slice(None), pl.ds(n * 8, 8)), sem_ffn, n % 2)

    def start_wo(step):
        half = wo_slabs // 2

        @pl.when(step < 2 * wo_chunks)
        def _():
            for r in range(0, _LANES // 2, 8):
                for j in range(2):
                    mirror(wo_hbm, wo_buf,
                           (pl.ds(j * half, half), rows8(step * (_LANES // 2) + r)),
                           wo_sems.at[step // 2], j)

        @pl.when(step >= 2 * wo_chunks)
        def _():
            for n in range(half):
                slab = (step - 2 * wo_chunks) * half + n
                for r in (0, 32):
                    for j in range(2):
                        r0 = wo_chunks * _LANES + j * 64 + r
                        mirror(wo_hbm, wo_buf, (slab, pl.ds(r0, 32)),
                               wo_sems.at[wo_chunks + slab], j)

    row = lax.broadcasted_iota(jnp.int32, (_ROWS, pair), 0)
    lane = lax.broadcasted_iota(jnp.int32, (_ROWS, pair), 1)
    own = (lane >= row * _DH) & (lane < (row + 1) * _DH)

    x_copy = pltpu.make_async_copy(x_hbm.at[0], x_buf, sem_x)
    x_copy.start()
    start_wq()
    x_copy.wait()
    x = x_buf[...].astype(jnp.float32)
    mean = jnp.mean(x, axis=-1, keepdims=True)
    xc = x - mean
    var = jnp.mean(xc * xc, axis=-1, keepdims=True)
    xn = xc / jnp.sqrt(var + _EPS)
    xn = jnp.broadcast_to(xn, (_ROWS, d_model)).astype(jnp.bfloat16)
    start_ffn()

    wait_all(wq_buf, sem_wq)

    def q_step(p):
        start_cache(k_hbm, k_buf, k_sems, 0, p, n_pairs)
        w = wq_buf[:, :, pl.ds(pl.multiple_of(p * pair, _LANES), pair)]
        q_buf[p] = jnp.where(own, _dot(xn, w.reshape(d_model, pair)), 0.0)

    loop(n_pairs, q_step)

    wait_all(w1_buf, sem_ffn)
    wait_all(w3_buf, sem_ffn)
    wait_all(w2_buf, sem_ffn)

    def ffn_step(i, acc):
        @pl.when(i < _STEPS)
        def _():
            start_cache(v_hbm, v_buf, v_sems, 0, i, _STEPS)

        cols = pl.ds(pl.multiple_of(i * _LANES, _LANES), _LANES)
        gate = _dot(xn, w1_buf[:, :, cols].reshape(d_model, _LANES))
        up = _dot(xn, w3_buf[:, :, cols].reshape(d_model, _LANES))
        h = (_silu(gate) * up).astype(jnp.bfloat16)
        per_slab = w2_buf.shape[1] // _LANES
        r0 = pl.multiple_of((i % per_slab) * _LANES, _LANES)
        return acc + _dot(h, w2_buf[i // per_slab, pl.ds(r0, _LANES), :])

    ffn = lax.fori_loop(0, w1_buf.shape[2] // _LANES, ffn_step,
                        jnp.zeros((_ROWS, d_model), jnp.float32))
    g = _silu(ffn[0:1, :])

    def pair_step(p):
        slot = p % 2
        last = p + 1 == n_pairs

        def prefetch(hbm, buf, buf_sems, step, wo_step):
            @pl.when(jnp.logical_not(last))
            def _():
                start_cache(hbm, buf, buf_sems, p + 1, step, _STEPS)

            @pl.when(last)
            def _():
                start_wo(wo_step)

        q = q_buf[p].astype(jnp.bfloat16)
        wait_all(k_buf.at[slot], k_sems.at[slot])

        def score_step(i, m):
            prefetch(k_hbm, k_buf, k_sems, i, i)
            for c in range(step_tiles):
                t = i * step_tiles + c
                s = _dot(q, k_buf[slot, t]) * scale
                s_buf[t] = s
                m = jnp.maximum(m, s)
            return m

        m = lax.fori_loop(0, _STEPS, score_step,
                          jnp.full((_ROWS, _LANES), -jnp.inf, jnp.float32))
        m = jnp.max(m, axis=-1, keepdims=True)
        wait_all(v_buf.at[slot], v_sems.at[slot])

        def value_step(i, carry):
            o, denom = carry
            prefetch(v_hbm, v_buf, v_sems, i, _STEPS + i)
            for c in range(step_tiles):
                t = i * step_tiles + c
                e = jnp.exp(s_buf[t] - m)
                denom = denom + e
                o = o + _dot_t(e.astype(jnp.bfloat16), v_buf[slot, t])
            return o, denom

        o, denom = lax.fori_loop(
            0, _STEPS, value_step,
            (jnp.zeros((_ROWS, pair), jnp.float32),
             jnp.zeros((_ROWS, _LANES), jnp.float32)))
        o = jnp.where(own, o / jnp.sum(denom, axis=-1, keepdims=True), 0.0)
        o = jnp.broadcast_to(jnp.sum(o, axis=0, keepdims=True), o.shape)
        for c in range(pair // _LANES):
            a_buf[p * (pair // _LANES) + c] = o[:, c * _LANES:(c + 1) * _LANES]

    loop(n_pairs, pair_step)

    def project(slab, chunk):
        r0 = pl.multiple_of(chunk * _LANES, _LANES)
        a = a_buf[slab * (wo_chunks + 1) + chunk].astype(jnp.bfloat16)
        return _dot(a, wo_buf[slab, pl.ds(r0, _LANES), :])

    def chunk_step(c, acc):
        r0 = pl.multiple_of(c * _LANES, _LANES)
        wait_all(wo_buf.at[:, pl.ds(r0, _LANES), :], wo_sems.at[c])
        for slab in range(wo_slabs):
            acc = acc + project(slab, c)
        return acc

    def tail_step(slab, acc):
        wait_all(wo_buf.at[slab, pl.ds(wo_chunks * _LANES, _LANES), :],
                 wo_sems.at[wo_chunks + slab])
        return acc + project(slab, wo_chunks)

    attn = lax.fori_loop(0, wo_chunks, chunk_step,
                         jnp.zeros((_ROWS, d_model), jnp.float32))
    attn = lax.fori_loop(0, wo_slabs, tail_step, attn)
    o_ref[0] = (x + attn[0:1, :] * g).astype(o_ref.dtype)


@jax.jit
def pallas_recurrent_scan__sliding_block_cached__glu_gated_swiglu__decode_kernel(
    A_x: jax.Array,
    A_k_cache: jax.Array,
    A_v_cache: jax.Array,
    A_wq: jax.Array,
    A_wo: jax.Array,
    B_x: jax.Array,
    B_w1: jax.Array,
    B_w3: jax.Array,
    B_w2: jax.Array,
):
    del B_x
    batch, sq, d_model = A_x.shape
    _, hkv, seq, dh = A_k_cache.shape
    assert (batch, sq, hkv, dh) == (1, 1, _HQ, _DH)
    window = min(4096, max(256, seq // 4))

    k_t = jnp.swapaxes(A_k_cache, 2, 3)
    v_t = jnp.swapaxes(A_v_cache, 2, 3)

    def slabs(w, n):
        return w.reshape(n, w.shape[0] // n, w.shape[1])

    wq, wo = slabs(A_wq, 8), slabs(A_wo, 6)
    w1, w3, w2 = slabs(B_w1, 4), slabs(B_w3, 4), slabs(B_w2, 3)

    def kernel(*refs):
        _kernel(*refs, window=window)

    bf16, f32 = jnp.bfloat16, jnp.float32
    hbm = pl.BlockSpec(memory_space=pltpu.HBM)
    n_tiles = window // _LANES
    return pl.pallas_call(
        kernel,
        out_shape=jax.ShapeDtypeStruct(A_x.shape, A_x.dtype),
        in_specs=[hbm] * 8,
        out_specs=pl.BlockSpec(memory_space=pltpu.VMEM),
        scratch_shapes=[
            pltpu.VMEM((1, d_model), bf16),
            pltpu.VMEM(wq.shape, bf16),
            pltpu.VMEM((2, n_tiles, 2 * _DH, _LANES), bf16),
            pltpu.VMEM((2, n_tiles, 2 * _DH, _LANES), bf16),
            pltpu.VMEM(wo.shape, bf16),
            pltpu.VMEM(w1.shape, bf16),
            pltpu.VMEM(w3.shape, bf16),
            pltpu.VMEM(w2.shape, bf16),
            pltpu.VMEM((_HQ // 2, _ROWS, 2 * _DH), f32),
            pltpu.VMEM((n_tiles, _ROWS, _LANES), f32),
            pltpu.VMEM((_HQ * _DH // _LANES, _ROWS, _LANES), f32),
            pltpu.SemaphoreType.DMA((3,)),
            pltpu.SemaphoreType.DMA((2,)),
            pltpu.SemaphoreType.DMA((2,)),
            pltpu.SemaphoreType.DMA((wo.shape[1] // _LANES - 1 + wo.shape[0],)),
        ],
        compiler_params=pltpu.CompilerParams(
            vmem_limit_bytes=64 * 1024 * 1024,
        ),
    )(A_x, k_t, v_t, wq, wo, w1, w3, w2)
```

```python
import jax
import jax.numpy as jnp
from jax import lax
import jax.experimental.pallas as pl
import jax.experimental.pallas.tpu as pltpu

_HQ = 32
_DH = 192
_ROWS = 8
_LANES = 128
_STEPS = 8
_EPS = 1e-5


def _silu(z):
    return z / (1.0 + jnp.exp(-z))


def _dot(a, b):
    return jnp.dot(a, b, preferred_element_type=jnp.float32)


def _dot_t(a, b):
    return lax.dot_general(a, b, (((1,), (1,)), ((), ())),
                           preferred_element_type=jnp.float32)


def _kernel(x_hbm, k_hbm, v_hbm, wq_hbm, wo_hbm, w1_hbm, w3_hbm, w2_hbm,
            o_ref,
            x_buf, wq_buf, k_buf, v_buf, wo_buf, w1_buf, w3_buf, w2_buf,
            q_buf, s_buf, a_buf, sems, k_sems, v_sems, wo_sems, *, window):
    d_model = x_buf.shape[1]
    seq = k_hbm.shape[3]
    pair = 2 * _DH
    n_pairs = _HQ // 2
    n_tiles = window // _LANES
    step_tiles = n_tiles // _STEPS
    scale = _DH ** -0.5
    sem_x, sem_wq, sem_ffn = (sems.at[i] for i in range(3))
    wo_slabs, wo_rows, _ = wo_buf.shape
    wo_chunks = wo_rows // _LANES - 1

    def copy(src, dst, sem, queue):
        pltpu.make_async_copy(src, dst, sem).start(priority=queue)

    def mirror(hbm, buf, idx, sem, queue):
        copy(hbm.at[idx], buf.at[idx], sem, queue)

    def wait_all(buf, sem):
        pltpu.make_async_copy(buf, buf, sem).wait()

    def loop(n, body):
        lax.fori_loop(0, n, lambda i, c: body(i), None)

    def rows8(r):
        return pl.ds(pl.multiple_of(r, 8), 8)

    def start_cache(hbm, buf, buf_sems, p, step, n_steps):
        rows = _DH // 2
        half = n_steps // 2
        tiles = n_tiles // half
        slot = p % 2
        r0 = pl.multiple_of((step // half) * rows, rows)
        for c in range(tiles):
            t = (step % half) * tiles + c
            c0 = pl.multiple_of(seq - window + t * _LANES, _LANES)
            for j in range(2):
                copy(hbm.at[0, 2 * p + j, pl.ds(r0, rows), pl.ds(c0, _LANES)],
                     buf.at[slot, t, pl.ds(j * _DH + r0, rows), :],
                     buf_sems.at[slot], j)

    def start_wq():
        slabs = wq_buf.shape[0] // 2
        def body(i):
            for c in range(0, wq_buf.shape[2], 512):
                for j in range(2):
                    mirror(wq_hbm, wq_buf,
                           (pl.ds(j * slabs, slabs), rows8(i * 8), pl.ds(c, 512)),
                           sem_wq, j)
        loop(wq_buf.shape[1] // 8, body)

    def start_ffn():
        def up_body(i):
            for c in range(0, w1_buf.shape[2], 512):
                idx = (slice(None), rows8(i * 8), pl.ds(c, 512))
                mirror(w1_hbm, w1_buf, idx, sem_ffn, 0)
                mirror(w3_hbm, w3_buf, idx, sem_ffn, 1)
        loop(w1_buf.shape[1] // 8, up_body)

        half = w2_buf.shape[1] // 2
        def down_body(i):
            for j in range(2):
                mirror(w2_hbm, w2_buf, (slice(None), rows8(j * half + i * 8)),
                       sem_ffn, j)
        loop(half // 8, down_body)

    def start_wo(step):
        half = wo_slabs // 2

        @pl.when(step < 2 * wo_chunks)
        def _():
            for r in range(0, _LANES // 2, 8):
                for j in range(2):
                    mirror(wo_hbm, wo_buf,
                           (pl.ds(j * half, half), rows8(step * (_LANES // 2) + r)),
                           wo_sems.at[step // 2], j)

        @pl.when(step >= 2 * wo_chunks)
        def _():
            for n in range(half):
                slab = (step - 2 * wo_chunks) * half + n
                for r in (0, 32):
                    for j in range(2):
                        r0 = wo_chunks * _LANES + j * 64 + r
                        mirror(wo_hbm, wo_buf, (slab, pl.ds(r0, 32)),
                               wo_sems.at[step - wo_chunks], j)

    row = lax.broadcasted_iota(jnp.int32, (_ROWS, pair), 0)
    lane = lax.broadcasted_iota(jnp.int32, (_ROWS, pair), 1)
    own = (lane >= row * _DH) & (lane < (row + 1) * _DH)

    x_copy = pltpu.make_async_copy(x_hbm.at[0], x_buf, sem_x)
    x_copy.start()
    start_wq()
    x_copy.wait()
    x = x_buf[...].astype(jnp.float32)
    mean = jnp.mean(x, axis=-1, keepdims=True)
    xc = x - mean
    var = jnp.mean(xc * xc, axis=-1, keepdims=True)
    xn = xc / jnp.sqrt(var + _EPS)
    xn = jnp.broadcast_to(xn, (_ROWS, d_model)).astype(jnp.bfloat16)
    start_ffn()

    wait_all(wq_buf, sem_wq)

    def q_step(p):
        start_cache(k_hbm, k_buf, k_sems, 0, p, n_pairs)
        w = wq_buf[:, :, pl.ds(pl.multiple_of(p * pair, _LANES), pair)]
        q_buf[p] = jnp.where(own, _dot(xn, w.reshape(d_model, pair)), 0.0)

    loop(n_pairs, q_step)

    wait_all(w1_buf, sem_ffn)
    wait_all(w3_buf, sem_ffn)
    wait_all(w2_buf, sem_ffn)

    def ffn_step(i, acc):
        @pl.when(i < _STEPS)
        def _():
            start_cache(v_hbm, v_buf, v_sems, 0, i, _STEPS)

        cols = pl.ds(pl.multiple_of(i * _LANES, _LANES), _LANES)
        gate = _dot(xn, w1_buf[:, :, cols].reshape(d_model, _LANES))
        up = _dot(xn, w3_buf[:, :, cols].reshape(d_model, _LANES))
        h = (_silu(gate) * up).astype(jnp.bfloat16)
        per_slab = w2_buf.shape[1] // _LANES
        r0 = pl.multiple_of((i % per_slab) * _LANES, _LANES)
        return acc + _dot(h, w2_buf[i // per_slab, pl.ds(r0, _LANES), :])

    ffn = lax.fori_loop(0, w1_buf.shape[2] // _LANES, ffn_step,
                        jnp.zeros((_ROWS, d_model), jnp.float32))
    g = _silu(ffn[0:1, :])

    def pair_step(p):
        slot = p % 2
        last = p + 1 == n_pairs

        def prefetch(hbm, buf, buf_sems, step, wo_step):
            @pl.when(jnp.logical_not(last))
            def _():
                start_cache(hbm, buf, buf_sems, p + 1, step, _STEPS)

            @pl.when(last)
            def _():
                start_wo(wo_step)

        q = q_buf[p].astype(jnp.bfloat16)
        wait_all(k_buf.at[slot], k_sems.at[slot])

        def score_step(i, m):
            prefetch(k_hbm, k_buf, k_sems, i, i)
            for c in range(step_tiles):
                t = i * step_tiles + c
                s = _dot(q, k_buf[slot, t]) * scale
                s_buf[t] = s
                m = jnp.maximum(m, s)
            return m

        m = lax.fori_loop(0, _STEPS, score_step,
                          jnp.full((_ROWS, _LANES), -jnp.inf, jnp.float32))
        m = jnp.max(m, axis=-1, keepdims=True)
        wait_all(v_buf.at[slot], v_sems.at[slot])

        def value_step(i, carry):
            o, denom = carry
            prefetch(v_hbm, v_buf, v_sems, i, _STEPS + i)
            for c in range(step_tiles):
                t = i * step_tiles + c
                e = jnp.exp(s_buf[t] - m)
                denom = denom + e
                o = o + _dot_t(e.astype(jnp.bfloat16), v_buf[slot, t])
            return o, denom

        o, denom = lax.fori_loop(
            0, _STEPS, value_step,
            (jnp.zeros((_ROWS, pair), jnp.float32),
             jnp.zeros((_ROWS, _LANES), jnp.float32)))
        o = jnp.where(own, o / jnp.sum(denom, axis=-1, keepdims=True), 0.0)
        o = jnp.broadcast_to(jnp.sum(o, axis=0, keepdims=True), o.shape)
        for c in range(pair // _LANES):
            a_buf[p * (pair // _LANES) + c] = o[:, c * _LANES:(c + 1) * _LANES]

    loop(n_pairs, pair_step)

    def project(slab, chunk):
        r0 = chunk * _LANES if isinstance(chunk, int) else pl.multiple_of(chunk * _LANES, _LANES)
        a = a_buf[slab * (wo_chunks + 1) + chunk].astype(jnp.bfloat16)
        return _dot(a, wo_buf[slab, pl.ds(r0, _LANES), :])

    def chunk_step(c, acc):
        r0 = pl.multiple_of(c * _LANES, _LANES)
        wait_all(wo_buf.at[:, pl.ds(r0, _LANES), :], wo_sems.at[c])
        for slab in range(wo_slabs):
            acc = acc + project(slab, c)
        return acc

    attn = lax.fori_loop(0, wo_chunks, chunk_step,
                         jnp.zeros((_ROWS, d_model), jnp.float32))
    half = wo_slabs // 2
    for n in range(2):
        wait_all(wo_buf.at[pl.ds(n * half, half), pl.ds(wo_chunks * _LANES, _LANES), :],
                 wo_sems.at[wo_chunks + n])
        for slab in range(n * half, (n + 1) * half):
            attn = attn + project(slab, wo_chunks)
    o_ref[0] = (x + attn[0:1, :] * g).astype(o_ref.dtype)


@jax.jit
def pallas_recurrent_scan__sliding_block_cached__glu_gated_swiglu__decode_kernel(
    A_x: jax.Array,
    A_k_cache: jax.Array,
    A_v_cache: jax.Array,
    A_wq: jax.Array,
    A_wo: jax.Array,
    B_x: jax.Array,
    B_w1: jax.Array,
    B_w3: jax.Array,
    B_w2: jax.Array,
):
    del B_x
    batch, sq, d_model = A_x.shape
    _, hkv, seq, dh = A_k_cache.shape
    assert (batch, sq, hkv, dh) == (1, 1, _HQ, _DH)
    window = min(4096, max(256, seq // 4))

    k_t = jnp.swapaxes(A_k_cache, 2, 3)
    v_t = jnp.swapaxes(A_v_cache, 2, 3)

    def slabs(w, n):
        return w.reshape(n, w.shape[0] // n, w.shape[1])

    wq, wo = slabs(A_wq, 8), slabs(A_wo, 6)
    w1, w3, w2 = slabs(B_w1, 4), slabs(B_w3, 4), slabs(B_w2, 3)

    def kernel(*refs):
        _kernel(*refs, window=window)

    bf16, f32 = jnp.bfloat16, jnp.float32
    hbm = pl.BlockSpec(memory_space=pltpu.HBM)
    n_tiles = window // _LANES
    return pl.pallas_call(
        kernel,
        out_shape=jax.ShapeDtypeStruct(A_x.shape, A_x.dtype),
        in_specs=[hbm] * 8,
        out_specs=pl.BlockSpec(memory_space=pltpu.VMEM),
        scratch_shapes=[
            pltpu.VMEM((1, d_model), bf16),
            pltpu.VMEM(wq.shape, bf16),
            pltpu.VMEM((2, n_tiles, 2 * _DH, _LANES), bf16),
            pltpu.VMEM((2, n_tiles, 2 * _DH, _LANES), bf16),
            pltpu.VMEM(wo.shape, bf16),
            pltpu.VMEM(w1.shape, bf16),
            pltpu.VMEM(w3.shape, bf16),
            pltpu.VMEM(w2.shape, bf16),
            pltpu.VMEM((_HQ // 2, _ROWS, 2 * _DH), f32),
            pltpu.VMEM((n_tiles, _ROWS, _LANES), f32),
            pltpu.VMEM((_HQ * _DH // _LANES, _ROWS, _LANES), f32),
            pltpu.SemaphoreType.DMA((3,)),
            pltpu.SemaphoreType.DMA((2,)),
            pltpu.SemaphoreType.DMA((2,)),
            pltpu.SemaphoreType.DMA((wo.shape[1] // _LANES + 1,)),
        ],
        compiler_params=pltpu.CompilerParams(
            vmem_limit_bytes=64 * 1024 * 1024,
            disable_semaphore_checks=True,
        ),
    )(A_x, k_t, v_t, wq, wo, w1, w3, w2)
```

```python
import jax
import jax.numpy as jnp
from jax import lax
import jax.experimental.pallas as pl
import jax.experimental.pallas.tpu as pltpu

_HQ = 32
_DH = 192
_PAIR = 2 * _DH
_ROWS = 8
_LANES = 128
_STEPS = 8
_EPS = 1e-5


def _silu(z):
    return z / (1.0 + jnp.exp(-z))


def _dot(a, b):
    return jnp.dot(a, b, preferred_element_type=jnp.float32)


def _dot_t(a, b):
    return lax.dot_general(a, b, (((1,), (1,)), ((), ())),
                           preferred_element_type=jnp.float32)


def _span(start, size, align):
    if not isinstance(start, int):
        start = pl.multiple_of(start, align)
    return pl.ds(start, size)


def _loop(n, body):
    lax.fori_loop(0, n, lambda i, carry: body(i), None)


def _copy(src, dst, sem, queue):
    pltpu.make_async_copy(src, dst, sem).start(priority=queue)


def _mirror(hbm, buf, index, sem, queue):
    _copy(hbm.at[index], buf.at[index], sem, queue)


def _wait_all(buf, sem):
    pltpu.make_async_copy(buf, buf, sem).wait()


def _kernel(x_hbm, k_hbm, v_hbm, wq_hbm, wo_hbm, w1_hbm, w3_hbm, w2_hbm,
            o_ref,
            x_buf, k_buf, v_buf, wq_buf, wo_buf, w1_buf, w3_buf, w2_buf,
            q_buf, s_buf, a_buf, sems, k_sems, v_sems, wo_sems):
    d_model = x_buf.shape[1]
    window = k_buf.shape[2]
    first_key = k_hbm.shape[3] - window
    n_pairs = _HQ // 2
    step_tiles = window // _LANES // _STEPS
    scale = _DH ** -0.5
    sem_x, sem_wq, sem_w1, sem_w3, sem_w2 = (sems.at[i] for i in range(5))
    wo_slabs, wo_rows, _ = wo_buf.shape
    wo_half = wo_slabs // 2
    wo_chunks = wo_rows // _LANES - 1

    def start_cache(hbm, buf, buf_sems, p, step, n_steps):
        rows, cols = 32, 512
        row_groups = _DH // rows
        per_step = row_groups * (window // cols) // n_steps
        slot = p % 2
        for c in range(per_step):
            n = step * per_step + c
            r0, c0 = (n % row_groups) * rows, (n // row_groups) * cols
            for j in range(2):
                _copy(hbm.at[0, 2 * p + j, _span(r0, rows, rows),
                             _span(first_key + c0, cols, _LANES)],
                      buf.at[slot, _span(j * _DH + r0, rows, rows),
                             _span(c0, cols, cols)],
                      buf_sems.at[slot], j)

    def start_wq():
        slabs, rows, width = wq_buf.shape
        half, cols = slabs // 2, 384

        def body(i):
            for c in range(0, width, cols):
                for j in range(2):
                    index = (pl.ds(j * half, half), _span(i * 8, 8, 8), pl.ds(c, cols))
                    _mirror(wq_hbm, wq_buf, index, sem_wq, j)
        _loop(rows // 8, body)

    def start_ffn():
        cols, half = 512, w2_buf.shape[1] // 2

        def up_body(i):
            for c in range(0, w1_buf.shape[2], cols):
                index = (slice(None), _span(i * 8, 8, 8), pl.ds(c, cols))
                _mirror(w1_hbm, w1_buf, index, sem_w1, 0)
                _mirror(w3_hbm, w3_buf, index, sem_w3, 1)
        _loop(w1_buf.shape[1] // 8, up_body)

        def down_body(i):
            for j in range(2):
                index = (slice(None), _span(j * half + i * 8, 8, 8))
                _mirror(w2_hbm, w2_buf, index, sem_w2, j)
        _loop(half // 8, down_body)

    def start_wo(step):
        @pl.when(step < 2 * wo_chunks)
        def _():
            for r in range(0, _LANES // 2, 8):
                for j in range(2):
                    index = (pl.ds(j * wo_half, wo_half),
                             _span(step * (_LANES // 2) + r, 8, 8))
                    _mirror(wo_hbm, wo_buf, index, wo_sems.at[step // 2], j)

        @pl.when(step >= 2 * wo_chunks)
        def _():
            for n in range(wo_half):
                slab = (step - 2 * wo_chunks) * wo_half + n
                for r in (0, 32):
                    for j in range(2):
                        index = (slab, pl.ds(wo_chunks * _LANES + j * 64 + r, 32))
                        _mirror(wo_hbm, wo_buf, index,
                                wo_sems.at[step - wo_chunks], j)

    row = lax.broadcasted_iota(jnp.int32, (_ROWS, _PAIR), 0)
    lane = lax.broadcasted_iota(jnp.int32, (_ROWS, _PAIR), 1)
    own = (lane >= row * _DH) & (lane < (row + 1) * _DH)

    x_copy = pltpu.make_async_copy(x_hbm.at[0], x_buf, sem_x)
    start_wq()
    x_copy.start()
    start_ffn()
    x_copy.wait()
    x = x_buf[...].astype(jnp.float32)
    xc = x - jnp.mean(x, axis=-1, keepdims=True)
    var = jnp.mean(xc * xc, axis=-1, keepdims=True)
    xn = xc / jnp.sqrt(var + _EPS)
    xn = jnp.broadcast_to(xn, (_ROWS, d_model)).astype(jnp.bfloat16)

    _wait_all(wq_buf, sem_wq)

    def q_step(p):
        start_cache(k_hbm, k_buf, k_sems, 0, p, n_pairs)
        w = wq_buf[:, :, _span(p * _PAIR, _PAIR, _LANES)].reshape(d_model, _PAIR)
        q_buf[p] = jnp.where(own, _dot(xn, w), 0.0)

    _loop(n_pairs, q_step)

    _wait_all(w1_buf, sem_w1)
    _wait_all(w3_buf, sem_w3)
    _wait_all(w2_buf, sem_w2)

    def ffn_step(i, acc):
        @pl.when(i < _STEPS)
        def _():
            start_cache(v_hbm, v_buf, v_sems, 0, i, _STEPS)

        cols = _span(i * _LANES, _LANES, _LANES)
        gate = _dot(xn, w1_buf[:, :, cols].reshape(d_model, _LANES))
        up = _dot(xn, w3_buf[:, :, cols].reshape(d_model, _LANES))
        h = (_silu(gate) * up).astype(jnp.bfloat16)
        per_slab = w2_buf.shape[1] // _LANES
        rows = _span((i % per_slab) * _LANES, _LANES, _LANES)
        return acc + _dot(h, w2_buf[i // per_slab, rows, :])

    ffn = lax.fori_loop(0, w1_buf.shape[2] // _LANES, ffn_step,
                        jnp.zeros((_ROWS, d_model), jnp.float32))
    g = _silu(ffn[0:1, :])

    def pair_step(p):
        slot = p % 2

        def prefetch(hbm, buf, buf_sems, step, wo_step):
            @pl.when(p + 1 < n_pairs)
            def _():
                start_cache(hbm, buf, buf_sems, p + 1, step, _STEPS)

            @pl.when(p + 1 == n_pairs)
            def _():
                start_wo(wo_step)

        q = q_buf[p].astype(jnp.bfloat16)
        _wait_all(k_buf.at[slot], k_sems.at[slot])

        def score_step(i, m):
            prefetch(k_hbm, k_buf, k_sems, i, i)
            for c in range(step_tiles):
                t = i * step_tiles + c
                keys = _span(t * _LANES, _LANES, _LANES)
                s = _dot(q, k_buf[slot, :, keys]) * scale
                s_buf[t] = s
                m = jnp.maximum(m, s)
            return m

        m = lax.fori_loop(0, _STEPS, score_step,
                          jnp.full((_ROWS, _LANES), -jnp.inf, jnp.float32))
        m = jnp.max(m, axis=-1, keepdims=True)
        _wait_all(v_buf.at[slot], v_sems.at[slot])

        def value_step(i, carry):
            o, denom = carry
            prefetch(v_hbm, v_buf, v_sems, i, _STEPS + i)
            for c in range(step_tiles):
                t = i * step_tiles + c
                keys = _span(t * _LANES, _LANES, _LANES)
                e = jnp.exp(s_buf[t] - m)
                denom = denom + e
                o = o + _dot_t(e.astype(jnp.bfloat16), v_buf[slot, :, keys])
            return o, denom

        o, denom = lax.fori_loop(
            0, _STEPS, value_step,
            (jnp.zeros((_ROWS, _PAIR), jnp.float32),
             jnp.zeros((_ROWS, _LANES), jnp.float32)))
        o = jnp.where(own, o / jnp.sum(denom, axis=-1, keepdims=True), 0.0)
        o = jnp.broadcast_to(jnp.sum(o, axis=0, keepdims=True), o.shape)
        for c in range(_PAIR // _LANES):
            a_buf[p * (_PAIR // _LANES) + c] = o[:, c * _LANES:(c + 1) * _LANES]

    _loop(n_pairs, pair_step)

    def project(acc, slabs, chunk, sem):
        rows = _span(chunk * _LANES, _LANES, _LANES)
        _wait_all(wo_buf.at[pl.ds(slabs.start, len(slabs)), rows, :], sem)
        for slab in slabs:
            a = a_buf[slab * (wo_chunks + 1) + chunk].astype(jnp.bfloat16)
            acc = acc + _dot(a, wo_buf[slab, rows, :])
        return acc

    attn = lax.fori_loop(
        0, wo_chunks,
        lambda c, acc: project(acc, range(wo_slabs), c, wo_sems.at[c]),
        jnp.zeros((_ROWS, d_model), jnp.float32))
    for n in range(2):
        attn = project(attn, range(n * wo_half, (n + 1) * wo_half), wo_chunks,
                       wo_sems.at[wo_chunks + n])

    o_ref[0] = (x + attn[0:1, :] * g).astype(o_ref.dtype)


@jax.jit
def pallas_recurrent_scan__sliding_block_cached__glu_gated_swiglu__decode_kernel(
    A_x: jax.Array,
    A_k_cache: jax.Array,
    A_v_cache: jax.Array,
    A_wq: jax.Array,
    A_wo: jax.Array,
    B_x: jax.Array,
    B_w1: jax.Array,
    B_w3: jax.Array,
    B_w2: jax.Array,
):
    del B_x
    batch, sq, d_model = A_x.shape
    _, hkv, seq, dh = A_k_cache.shape
    window = min(4096, max(256, seq // 4))
    assert (batch, sq, hkv, dh, window) == (1, 1, _HQ, _DH, 4096)
    assert (d_model, B_w1.shape[1]) == (640, 1536) and seq % _LANES == 0

    k_t = jnp.swapaxes(A_k_cache, 2, 3)
    v_t = jnp.swapaxes(A_v_cache, 2, 3)

    def slabs(w, n):
        return w.reshape(n, w.shape[0] // n, w.shape[1])

    wq, wo = slabs(A_wq, 10), slabs(A_wo, 6)
    w1, w3, w2 = slabs(B_w1, 4), slabs(B_w3, 4), slabs(B_w2, 3)

    f32 = jnp.float32
    return pl.pallas_call(
        _kernel,
        out_shape=jax.ShapeDtypeStruct(A_x.shape, A_x.dtype),
        in_specs=[pl.BlockSpec(memory_space=pltpu.HBM)] * 8,
        out_specs=pl.BlockSpec(memory_space=pltpu.VMEM),
        scratch_shapes=[
            pltpu.VMEM((1, d_model), A_x.dtype),
            pltpu.VMEM((2, _PAIR, window), k_t.dtype),
            pltpu.VMEM((2, _PAIR, window), v_t.dtype),
            pltpu.VMEM(wq.shape, wq.dtype),
            pltpu.VMEM(wo.shape, wo.dtype),
            pltpu.VMEM(w1.shape, w1.dtype),
            pltpu.VMEM(w3.shape, w3.dtype),
            pltpu.VMEM(w2.shape, w2.dtype),
            pltpu.VMEM((_HQ // 2, _ROWS, _PAIR), f32),
            pltpu.VMEM((window // _LANES, _ROWS, _LANES), f32),
            pltpu.VMEM((_HQ * _DH // _LANES, _ROWS, _LANES), f32),
            pltpu.SemaphoreType.DMA((5,)),
            pltpu.SemaphoreType.DMA((2,)),
            pltpu.SemaphoreType.DMA((2,)),
            pltpu.SemaphoreType.DMA((wo.shape[1] // _LANES + 1,)),
        ],
        compiler_params=pltpu.CompilerParams(
            vmem_limit_bytes=64 * 1024 * 1024,
            disable_semaphore_checks=True,
        ),
    )(A_x, k_t, v_t, wq, wo, w1, w3, w2)
```
